```python
import os as _os
_os.environ.setdefault("JAX_PLATFORMS", "cpu")
import jax
import jax.numpy as jnp

def _softmax(x, axis=-1):
    return jax.nn.softmax(x, axis=axis)
def _gelu(x):
    return jax.nn.gelu(x, approximate=True)
def _silu(x):
    return jax.nn.silu(x)
def _sigmoid(x):
    return jax.nn.sigmoid(x)
def _layernorm(x, axis=-1, eps=1e-5):
    m = jnp.mean(x, axis=axis, keepdims=True)
    v = jnp.var(x, axis=axis, keepdims=True)
    return (x - m) / jnp.sqrt(v + eps)
def _scatter_add(tgt, idx, src, axis=0):
    return tgt.at[idx].add(src)
def _segment_sum(src, seg, n):
    return jax.ops.segment_sum(src, seg, n)
class _Rng:
    def __init__(self, key):
        self._k = key
    def _next(self):
        self._k, sub = jax.random.split(self._k)
        return sub
    def normal(self, shape):
        return jax.random.normal(self._next(), shape, dtype=jnp.bfloat16)
    def randint(self, lo, hi, shape):
        return jax.random.randint(self._next(), shape, lo, hi, dtype=jnp.int32)
    def uniform(self, shape, lo=0.0, hi=1.0):
        return jax.random.uniform(self._next(), shape, jnp.bfloat16, lo, hi)
    def permutation(self, n):
        return jax.random.permutation(self._next(), n)


kernel_name = 'gated_mix__grouped_kv_mqa__glu_gated_reglu__prompt'

def setup_inputs():
    _rng = _Rng(jax.random.key(int.from_bytes(__import__("os").urandom(4), "little")))
    _w = (lambda a: (lambda t: t.astype(jnp.bfloat16) if jnp.issubdtype(t.dtype, jnp.floating) else t)(jnp.asarray(a)))
    def _A_setup():
        B, S, D, H = 1, 2048, 640, 32
        Dh = D // H
        return {
            "x": _w((lambda *s: _rng.normal(s) * 0.05)(B, S, D)),
            "wq": _w((lambda *s: _rng.normal(s) * 0.2)(D, H * Dh)),
            "wk": _w((lambda *s: _rng.normal(s) * 0.2)(D, Dh)),
            "wv": _w((lambda *s: _rng.normal(s) * 0.05)(D, Dh)),
            "wo": _w((lambda *s: _rng.normal(s) * 0.05)(H * Dh, D)),
        }
    _A_in = _A_setup()

    def _B_setup():
        B, S, D, F = 1, 2048, 640, 1536
        return {
            "x": _w((lambda *s: _rng.normal(s) * 0.05)(B, S, D)),
            "W_gate": _w((lambda *s: _rng.normal(s) * 0.4)(D, F) * (2.0 / D) ** 0.5),
            "W_up": _w((lambda *s: _rng.normal(s) * 0.4)(D, F) * (2.0 / D) ** 0.5),
            "W_down": _w((lambda *s: _rng.normal(s) * 0.4)(F, D) * (1.0 / F) ** 0.5),
        }
    _B_in = _B_setup()

    return {
        "A_x": _A_in["x"],
        "A_wq": _A_in["wq"],
        "A_wk": _A_in["wk"],
        "A_wv": _A_in["wv"],
        "A_wo": _A_in["wo"],
        "B_x": _B_in["x"],
        "B_W_gate": _B_in["W_gate"],
        "B_W_up": _B_in["W_up"],
        "B_W_down": _B_in["W_down"],
        "gate_w": _w((lambda *s: _rng.normal(s) * 0.05)(640) * 16.0),
    }

def reference(A_x, A_wq, A_wk, A_wv, A_wo, B_x, B_W_gate, B_W_up, B_W_down, gate_w):
    def _A_ref(x, wq, wk, wv, wo):
        B, S, D = x.shape
        H = 32
        Dh = D // H
        q = (lambda x, *d: x.transpose(*d))((x @ wq).reshape(B, S, H, Dh), 0, 2, 1, 3)
        k = x @ wk
        v = x @ wv
        scores = jnp.einsum("bhqd,bkd->bhqk", q, k) * (Dh ** -0.5)
        p = _softmax(scores, axis=-1)
        o = jnp.einsum("bhqk,bkd->bhqd", p, v)
        return (lambda x, *d: x.transpose(*d))(o, 0, 2, 1, 3).reshape(B, S, H * Dh) @ wo

    def _B_ref(x, W_gate, W_up, W_down):
        gate = jnp.einsum("bsd,df->bsf", x, W_gate)
        up = jnp.einsum("bsd,df->bsf", x, W_up)
        gate = gate * (lambda x, dt: x.astype(dt))(gate > 0, gate.dtype)
        h = gate * up
        return jnp.einsum("bsf,fd->bsd", h, W_down)

    x = A_x
    g = _sigmoid((x * gate_w).sum(-1, keepdims=True))
    a = _A_ref(x, A_wq, A_wk, A_wv, A_wo)
    b = _B_ref(x, B_W_gate, B_W_up, B_W_down)
    return g * a + (1 - g) * b
```

```python
import jax
import jax.numpy as jnp
from jax import lax
from jax.experimental import pallas as pl
from jax.experimental.pallas import tpu as pltpu

S = 2048
D = 640
H = 32
DH = 20
F = 1536
TQ = 512
CK = 128
NCK = S // CK
NP = H // 2
KD = 48
VR = 24
FC = 512
LOG2E = 1.4426950408889634
QSCALE = (DH ** -0.5) * LOG2E
SAFE_M = 16.0

F32 = jnp.float32
BF16 = jnp.bfloat16


def _dot(a, b):
    return jnp.dot(a, b, preferred_element_type=F32)


def _kernel(x_ref, wq_ref, wk_ref, wv_ref, wo_ref, wg_ref, wu_ref, wd_ref, gw_ref,
            o_ref,
            ke_ref, ko_ref, vt_ref, qw_ref, pa_ref, pb_ref, ot_ref, kn_ref, flag_ref):
    step = pl.program_id(0)
    nsteps = pl.num_programs(0)

    def qproj(blk):
        r0 = pl.multiple_of(blk * TQ, TQ)
        xb = x_ref[pl.ds(r0, TQ), :]
        q = _dot(xb, wq_ref[...]) * QSCALE
        qt = q.T
        sq = (qt * qt).astype(BF16)
        hrow = lax.broadcasted_iota(jnp.int32, (H, D), 0)
        hcol = lax.broadcasted_iota(jnp.int32, (H, D), 1)
        e = jnp.logical_and(hcol >= hrow * DH, hcol < (hrow + 1) * DH)
        hs = _dot(jnp.where(e, 1.0, 0.0).astype(BF16), sq)
        m2 = jnp.max(hs) * kn_ref[0] * 1.05
        safe = m2 <= SAFE_M * SAFE_M
        flag_ref[0] = safe.astype(jnp.int32)
        mval = jnp.where(safe, -jnp.sqrt(jnp.full((8, TQ), m2, F32)), 0.0)
        srow = lax.broadcasted_iota(jnp.int32, (8, TQ), 0)
        mt = jnp.where(srow < 2, mval, 0.0)
        qw = jnp.concatenate(
            [qt.reshape(NP, 2 * DH, TQ), jnp.broadcast_to(mt[None], (NP, 8, TQ))], axis=1)
        qw_ref[...] = qw.astype(BF16)

    @pl.when(step == 0)
    def _init():
        pb_ref[...] = jnp.ones_like(pb_ref)
        zpad = jnp.zeros((D, 128 - DH), F32)
        wkp = jnp.concatenate([wk_ref[...].astype(F32), zpad], axis=1)
        wvp = jnp.concatenate([wv_ref[...].astype(F32), zpad], axis=1)
        wall = wkp + pltpu.roll(wkp, DH, 1) + pltpu.roll(wvp, 64, 1)
        r = _dot(x_ref[...], wall.astype(BF16))
        r = r.astype(BF16).astype(F32)
        lane = lax.broadcasted_iota(jnp.int32, (S, 128), 1)
        kev = jnp.where(lane < DH, r, 0.0)
        kn_ref[0] = jnp.max(jnp.sum(kev * kev, axis=1, keepdims=True))
        ke_ref[...] = jnp.where(lane == 2 * DH, 1.0, kev).astype(BF16)
        kod = jnp.where(jnp.logical_and(lane >= DH, lane < 2 * DH), r, 0.0)
        ko_ref[...] = jnp.where(lane == 2 * DH + 1, 1.0, kod).astype(BF16)
        rt = r.T
        vrow = lax.broadcasted_iota(jnp.int32, (VR, S), 0)
        vt_ref[...] = jnp.where(vrow < DH, rt[64:64 + VR, :],
                                jnp.where(vrow == DH, 1.0, 0.0))
        qproj(0)

    def finish(acc):
        return acc[0:DH, :] * (1.0 / acc[DH:DH + 1, :])

    def pv(p_r):
        acc = None
        for c in range(NCK):
            o = _dot(vt_ref[:, c * CK:(c + 1) * CK], p_r[c * CK:(c + 1) * CK, :])
            acc = o if acc is None else acc + o
        return acc

    @pl.when(flag_ref[0] == 1)
    def _fast():
        def stage(k_ref, qw, p_w, p_r):
            acc = None
            for c in range(NCK):
                s = _dot(k_ref[c * CK:(c + 1) * CK, 0:KD], qw)
                p_w[c * CK:(c + 1) * CK, :] = jnp.exp2(s)
                o = _dot(vt_ref[:, c * CK:(c + 1) * CK], p_r[c * CK:(c + 1) * CK, :])
                acc = o if acc is None else acc + o
            return acc

        def body(j, carry):
            qw = qw_ref[j]
            accb = stage(ke_ref, qw, pa_ref, pb_ref)
            ot_ref[j, DH:2 * DH, :] = finish(accb)
            acca = stage(ko_ref, qw, pb_ref, pa_ref)
            ot_ref[j + 1, 0:DH, :] = finish(acca)
            return carry

        lax.fori_loop(0, NP, body, 0)

    @pl.when(flag_ref[0] != 1)
    def _slow():
        def probs(k_ref, qw, p_w):
            m = None
            for c in range(NCK):
                s = _dot(k_ref[c * CK:(c + 1) * CK, 0:KD], qw)
                p_w[c * CK:(c + 1) * CK, :] = s
                mc = jnp.max(s, axis=0, keepdims=True)
                m = mc if m is None else jnp.maximum(m, mc)
            for c in range(NCK):
                p_w[c * CK:(c + 1) * CK, :] = jnp.exp2(p_w[c * CK:(c + 1) * CK, :] - m)

        def body(j, carry):
            qw = qw_ref[j]
            probs(ke_ref, qw, pa_ref)
            ot_ref[j + 1, 0:DH, :] = finish(pv(pa_ref))
            probs(ko_ref, qw, pb_ref)
            ot_ref[j + 1, DH:2 * DH, :] = finish(pv(pb_ref))
            return carry

        lax.fori_loop(0, NP, body, 0)

    ot_ref[NP, DH:2 * DH, :] = finish(pv(pb_ref))
    ot = ot_ref[1:NP + 1].reshape(D, TQ)
    a = _dot(ot.T.astype(BF16), wo_ref[...])

    r0 = pl.multiple_of(step * TQ, TQ)
    xb = x_ref[pl.ds(r0, TQ), :]
    b = None
    for fc in range(F // FC):
        gt = _dot(xb, wg_ref[:, fc * FC:(fc + 1) * FC])
        up = _dot(xb, wu_ref[:, fc * FC:(fc + 1) * FC])
        h = (jnp.maximum(gt, 0.0) * up).astype(BF16)
        bb = _dot(h, wd_ref[fc * FC:(fc + 1) * FC, :])
        b = bb if b is None else b + bb

    logit = jnp.sum(xb.astype(F32) * gw_ref[...].astype(F32), axis=1, keepdims=True)
    g = 1.0 / (1.0 + jnp.exp(-logit))
    o_ref[0] = (g * a + (1.0 - g) * b).astype(o_ref.dtype)

    qproj(jnp.minimum(step + 1, nsteps - 1))


@jax.jit
def pallas_gated_mix__grouped_kv_mqa__glu_gated_reglu__prompt_kernel(
    A_x: jax.Array,
    A_wq: jax.Array,
    A_wk: jax.Array,
    A_wv: jax.Array,
    A_wo: jax.Array,
    B_x: jax.Array,
    B_W_gate: jax.Array,
    B_W_up: jax.Array,
    B_W_down: jax.Array,
    gate_w: jax.Array,
):
    x = A_x.reshape(S, D)
    gw = gate_w.reshape(1, D)

    def full(shape):
        return pl.BlockSpec(shape, lambda i: (0,) * len(shape))

    return pl.pallas_call(
        _kernel,
        grid=(S // TQ,),
        in_specs=[
            full((S, D)), full((D, D)), full((D, DH)), full((D, DH)), full((D, D)),
            full((D, F)), full((D, F)), full((F, D)), full((1, D)),
        ],
        out_specs=pl.BlockSpec((1, TQ, D), lambda i: (0, i, 0)),
        out_shape=jax.ShapeDtypeStruct((1, S, D), BF16),
        scratch_shapes=[
            pltpu.VMEM((S, 128), BF16),
            pltpu.VMEM((S, 128), BF16),
            pltpu.VMEM((VR, S), F32),
            pltpu.VMEM((NP, KD, TQ), BF16),
            pltpu.VMEM((S, TQ), F32),
            pltpu.VMEM((S, TQ), F32),
            pltpu.VMEM((NP + 1, 2 * DH, TQ), F32),
            pltpu.SMEM((1,), F32),
            pltpu.SMEM((1,), jnp.int32),
        ],
        compiler_params=pltpu.CompilerParams(
            dimension_semantics=("arbitrary",),
            vmem_limit_bytes=100 * 1024 * 1024,
        ),
    )(x, A_wq, A_wk, A_wv, A_wo, B_W_gate, B_W_up, B_W_down, gw)
```

```python
import jax
import jax.numpy as jnp
from jax import lax
from jax.experimental import pallas as pl
from jax.experimental.pallas import tpu as pltpu

S = 2048
D = 640
H = 32
DH = 20
F = 1536
TQ = 512
NBLK = S // TQ
CK = 128
NCK = S // CK
NP = H // 2
UNROLL = 4
KD = 48
VR = 24
FC = 512
LOG2E = 1.4426950408889634
QSCALE = (DH ** -0.5) * LOG2E
SAFE_M = 16.0

F32 = jnp.float32
BF16 = jnp.bfloat16


def _dot(a, b):
    return jnp.dot(a, b, preferred_element_type=F32)


def _rev8(p):
    n = p.shape[0] // 8
    return jnp.concatenate([p[8 * (n - 1 - t):8 * (n - t)] for t in range(n)], axis=0)


def _kernel(x_hbm, wq_hbm, wkt_hbm, wvt_hbm, wo_hbm, wg_hbm, wu_hbm, wd_hbm, gw_hbm,
            o_ref,
            x_ref, wq_ref, wkt_ref, wvt_ref, wo_ref, wg_ref, wu_ref, wd_ref, gw_ref,
            ke_ref, ko_ref, vt_ref, qw_ref, carry_ref, ot_ref, wt_ref,
            kn_ref, flag_ref, sems):
    step = pl.program_id(0)

    def x_copy(c):
        return pltpu.make_async_copy(x_hbm.at[pl.ds(c * TQ, TQ)],
                                     x_ref.at[pl.ds(c * TQ, TQ)], sems.at[c])

    early = [pltpu.make_async_copy(wq_hbm, wq_ref, sems.at[NBLK]),
             pltpu.make_async_copy(wkt_hbm, wkt_ref, sems.at[NBLK + 1]),
             pltpu.make_async_copy(wvt_hbm, wvt_ref, sems.at[NBLK + 2])]
    late = [pltpu.make_async_copy(wo_hbm, wo_ref, sems.at[NBLK + 3]),
            pltpu.make_async_copy(wg_hbm, wg_ref, sems.at[NBLK + 4]),
            pltpu.make_async_copy(wu_hbm, wu_ref, sems.at[NBLK + 5]),
            pltpu.make_async_copy(wd_hbm, wd_ref, sems.at[NBLK + 6]),
            pltpu.make_async_copy(gw_hbm, gw_ref, sems.at[NBLK + 7])]

    def probs(j, par, c):
        k_ref = ko_ref if par else ke_ref
        s = _dot(k_ref[c * CK:(c + 1) * CK, 0:KD], qw_ref[j])
        return _rev8(jnp.exp2(s))

    def q_raw(blk):
        r0 = pl.multiple_of(blk * TQ, TQ)
        xb = x_ref[pl.ds(r0, TQ), :]
        q = _dot(xb, wq_ref[...]) * QSCALE
        return q.T

    def q_finish(qt):
        sq = (qt * qt).astype(BF16)
        hrow = lax.broadcasted_iota(jnp.int32, (H, D), 0)
        hcol = lax.broadcasted_iota(jnp.int32, (H, D), 1)
        e = jnp.logical_and(hcol >= hrow * DH, hcol < (hrow + 1) * DH)
        hs = _dot(jnp.where(e, 1.0, 0.0).astype(BF16), sq)
        m2 = jnp.max(hs) * kn_ref[0] * 1.05
        safe = m2 <= SAFE_M * SAFE_M
        flag_ref[0] = safe.astype(jnp.int32)
        mval = jnp.where(safe, -jnp.sqrt(jnp.full((8, TQ), m2, F32)), 0.0)
        srow = lax.broadcasted_iota(jnp.int32, (8, TQ), 0)
        mt = jnp.where(srow < 2, mval, 0.0)
        qw = jnp.concatenate(
            [qt.reshape(NP, 2 * DH, TQ), jnp.broadcast_to(mt[None], (NP, 8, TQ))], axis=1)
        qw_ref[...] = qw.astype(BF16)
        carry_ref[...] = probs(0, 0, 0)

    @pl.when(step == 0)
    def _init():
        early[1].start()
        early[2].start()
        x_copy(0).start()
        early[0].start()
        for c in range(1, NBLK):
            x_copy(c).start()
        wt_ref[...] = jnp.zeros_like(wt_ref)
        early[1].wait()
        early[2].wait()
        wt_ref[0:DH, :] = wkt_ref[...].astype(F32)
        wt_ref[DH:2 * DH, :] = wkt_ref[...].astype(F32)
        wt_ref[64:64 + DH, :] = wvt_ref[...].astype(F32)
        wall = wt_ref[...].T.astype(BF16)
        lane = lax.broadcasted_iota(jnp.int32, (TQ, 128), 1)
        vrow = lax.broadcasted_iota(jnp.int32, (VR, CK), 0)
        ke_fill = jnp.where(lane == 2 * DH, 1.0, 0.0)
        ko_fill = jnp.where(lane == 2 * DH + 1, 1.0, 0.0)

        def kv(c, kn):
            rows = slice(c * TQ, (c + 1) * TQ)
            r = _dot(x_ref[rows, :], wall)
            r = r.astype(BF16).astype(F32)
            ke_ref[rows, :] = jnp.where(lane < DH, r, ke_fill).astype(BF16)
            ko_ref[rows, :] = jnp.where(
                jnp.logical_and(lane >= DH, lane < 2 * DH), r, ko_fill).astype(BF16)
            for t in range(TQ // CK):
                rt = _rev8(r[t * CK:(t + 1) * CK, :]).T
                col = c * TQ + t * CK
                vt_ref[:, col:col + CK] = jnp.where(
                    vrow < DH, rt[64:64 + VR, :], jnp.where(vrow == DH, 1.0, 0.0))
                kt = rt[0:DH, :]
                n2 = jnp.sum(kt * kt, axis=0, keepdims=True)
                kn = n2 if kn is None else jnp.maximum(kn, n2)
            return kn

        x_copy(0).wait()
        early[0].wait()
        kn = kv(0, None)
        qt = q_raw(0)
        for c in range(1, NBLK):
            x_copy(c).wait()
        for cp in late:
            cp.start()
        for c in range(1, NBLK):
            kn = kv(c, kn)
        kn_ref[0] = jnp.max(kn)
        q_finish(qt)

    def finish(acc):
        return acc[0:DH, :] * (1.0 / acc[DH:DH + 1, :])

    @pl.when(flag_ref[0] == 1)
    def _fast():
        def body(i, carry):
            j0 = i * UNROLL
            pend = carry_ref[...]
            acc = None
            n = UNROLL * 2 * NCK
            for g in range(n):
                gq = g + 1
                if gq < n:
                    nxt = probs(j0 + gq // (2 * NCK), (gq // NCK) % 2, gq % NCK)
                else:
                    nxt = probs(jnp.minimum(j0 + UNROLL, NP - 1), 0, 0)
                c = g % NCK
                o = _dot(vt_ref[:, c * CK:(c + 1) * CK], pend)
                acc = o if c == 0 else acc + o
                if c == NCK - 1:
                    par = (g // NCK) % 2
                    ot_ref[j0 + g // (2 * NCK), par * DH:(par + 1) * DH, :] = finish(acc)
                pend = nxt
            carry_ref[...] = pend
            return carry

        lax.fori_loop(0, NP // UNROLL, body, 0)

    @pl.when(flag_ref[0] != 1)
    def _slow():
        def head(j, par, s_ref):
            k_ref = ko_ref if par else ke_ref
            qw = qw_ref[j]
            m = None
            for c in range(NCK):
                s = _dot(k_ref[c * CK:(c + 1) * CK, 0:KD], qw)
                s_ref[c * CK:(c + 1) * CK, :] = s
                mc = jnp.max(s, axis=0, keepdims=True)
                m = mc if m is None else jnp.maximum(m, mc)
            acc = None
            for c in range(NCK):
                p = _rev8(jnp.exp2(s_ref[c * CK:(c + 1) * CK, :] - m))
                o = _dot(vt_ref[:, c * CK:(c + 1) * CK], p)
                acc = o if acc is None else acc + o
            ot_ref[j, par * DH:(par + 1) * DH, :] = finish(acc)

        def scoped(s_ref):
            def body(j, carry):
                head(j, 0, s_ref)
                head(j, 1, s_ref)
                return carry
            lax.fori_loop(0, NP, body, 0)

        pl.run_scoped(scoped, pltpu.VMEM((S, TQ), F32))

    @pl.when(step == 0)
    def _wait_late():
        for cp in late:
            cp.wait()

    def epilogue(next_q):
        if next_q:
            qt = q_raw(jnp.minimum(step + 1, NBLK - 1))
        ot = ot_ref[...].reshape(D, TQ)
        a = _dot(ot.T.astype(BF16), wo_ref[...])
        if next_q:
            q_finish(qt)
        r0 = pl.multiple_of(step * TQ, TQ)
        xb = x_ref[pl.ds(r0, TQ), :]
        b = None
        for fc in range(F // FC):
            gt = _dot(xb, wg_ref[:, fc * FC:(fc + 1) * FC])
            up = _dot(xb, wu_ref[:, fc * FC:(fc + 1) * FC])
            h = (jnp.maximum(gt, 0.0) * up).astype(BF16)
            bb = _dot(h, wd_ref[fc * FC:(fc + 1) * FC, :])
            b = bb if b is None else b + bb
        logit = jnp.sum(xb.astype(F32) * gw_ref[...].astype(F32).reshape(1, D), axis=1, keepdims=True)
        g = 1.0 / (1.0 + jnp.exp(-logit))
        o_ref[0] = (g * a + (1.0 - g) * b).astype(o_ref.dtype)

    epilogue(True)


@jax.jit
def pallas_gated_mix__grouped_kv_mqa__glu_gated_reglu__prompt_kernel(
    A_x: jax.Array,
    A_wq: jax.Array,
    A_wk: jax.Array,
    A_wv: jax.Array,
    A_wo: jax.Array,
    B_x: jax.Array,
    B_W_gate: jax.Array,
    B_W_up: jax.Array,
    B_W_down: jax.Array,
    gate_w: jax.Array,
):
    x = A_x.reshape(S, D)
    gw = gate_w
    hbm = pl.BlockSpec(memory_space=pl.ANY)

    return pl.pallas_call(
        _kernel,
        grid=(NBLK,),
        in_specs=[hbm] * 9,
        out_specs=pl.BlockSpec((1, TQ, D), lambda i: (0, i, 0)),
        out_shape=jax.ShapeDtypeStruct((1, S, D), BF16),
        scratch_shapes=[
            pltpu.VMEM((S, D), BF16),
            pltpu.VMEM((D, D), BF16),
            pltpu.VMEM((DH, D), BF16),
            pltpu.VMEM((DH, D), BF16),
            pltpu.VMEM((D, D), BF16),
            pltpu.VMEM((D, F), BF16),
            pltpu.VMEM((D, F), BF16),
            pltpu.VMEM((F, D), BF16),
            pltpu.VMEM((D,), BF16),
            pltpu.VMEM((S, 128), BF16),
            pltpu.VMEM((S, 128), BF16),
            pltpu.VMEM((VR, S), F32),
            pltpu.VMEM((NP, KD, TQ), BF16),
            pltpu.VMEM((CK, TQ), F32),
            pltpu.VMEM((NP, 2 * DH, TQ), F32),
            pltpu.VMEM((128, D), F32),
            pltpu.SMEM((1,), F32),
            pltpu.SMEM((1,), jnp.int32),
            pltpu.SemaphoreType.DMA((NBLK + 8,)),
        ],
        compiler_params=pltpu.CompilerParams(
            dimension_semantics=("arbitrary",),
            vmem_limit_bytes=100 * 1024 * 1024,
        ),
    )(x, A_wq, A_wk.T, A_wv.T, A_wo, B_W_gate, B_W_up, B_W_down, gw)
```

```python
import jax
import jax.numpy as jnp
from jax import lax
from jax.experimental import pallas as pl
from jax.experimental.pallas import tpu as pltpu

S = 2048
D = 640
H = 32
DH = 20
F = 1536
TQ = 512
NBLK = S // TQ
CK = 128
NCK = S // CK
SC = 256
NSC = S // SC
VR_K = 16
MR_K = SC - VR_K
GL = 256
NP = H // 2
UNROLL = 4
KD = 32
VR = 24
FC = 512
LOG2E = 1.4426950408889634
QSCALE = (DH ** -0.5) * LOG2E
SAFE_M = 16.0

NZ = 64
F32 = jnp.float32
BF16 = jnp.bfloat16


def _dot(a, b):
    return jnp.dot(a, b, preferred_element_type=F32)


def _rev8(p):
    n = p.shape[0] // 8
    return jnp.concatenate([p[8 * (n - 1 - t):8 * (n - t)] for t in range(n)], axis=0)


def _kernel(x_hbm, wq_hbm, wkt_hbm, wvt_hbm, wo_hbm, wg_hbm, wu_hbm, wd_hbm, gw_hbm,
            o_ref,
            x_ref, wq_ref, wkt_ref, wvt_ref, wo_ref, wg_ref, wu_ref, wd_ref, gw_ref,
            ke_ref, vt_ref, qw_ref, carry_ref, ot_ref, wt_ref, qt_ref,
            kb_ref, qb_ref, kn_ref, m_ref, flag_ref, z_ref, sems):
    step = pl.program_id(0)

    def x_copy(c):
        return pltpu.make_async_copy(x_hbm.at[pl.ds(c * TQ, TQ)],
                                     x_ref.at[pl.ds(c * TQ, TQ)], sems.at[c])

    early = [pltpu.make_async_copy(wq_hbm, wq_ref, sems.at[NBLK]),
             pltpu.make_async_copy(wkt_hbm, wkt_ref, sems.at[NBLK + 1]),
             pltpu.make_async_copy(wvt_hbm, wvt_ref, sems.at[NBLK + 2])]
    late = [pltpu.make_async_copy(wo_hbm, wo_ref, sems.at[NBLK + 3]),
            pltpu.make_async_copy(wg_hbm, wg_ref, sems.at[NBLK + 4]),
            pltpu.make_async_copy(wu_hbm, wu_ref, sems.at[NBLK + 5]),
            pltpu.make_async_copy(wd_hbm, wd_ref, sems.at[NBLK + 6]),
            pltpu.make_async_copy(gw_hbm, gw_ref, sems.at[NBLK + 7])]

    def q_bcast(j, par):
        return [jnp.broadcast_to(qb_ref[j, par * DH + d:par * DH + d + 1, :], (8, TQ))
                for d in range(DH)]

    def probs(j, par, c, g, qbs):
        s = _dot(ke_ref[c * SC:c * SC + MR_K, 0:KD], qw_ref[j + z_ref[g % NZ], par])
        lanes = []
        for ll in range(TQ // GL):
            zi = z_ref[(g * (TQ // GL) + ll + 7) % NZ]
            a = jnp.full((VR_K, GL), m_ref[0], F32)
            for d in range(DH):
                kb = kb_ref[d + zi, c * VR_K:(c + 1) * VR_K, :]
                kb = jnp.concatenate([kb] * (GL // 128), axis=1)
                qb = qbs[d][:, ll * GL:(ll + 1) * GL]
                qb = jnp.concatenate([qb] * (VR_K // 8), axis=0)
                a = a + kb * qb
            parts = [a[rr * 8:(rr + 1) * 8, lq * 128:(lq + 1) * 128]
                     for rr in range(VR_K // 8) for lq in range(GL // 128)]
            t = parts[0]
            for part in parts[1:]:
                t = t + part
            t = t * 0.0
            t = jnp.concatenate([t] * (GL // 128), axis=1)
            t = jnp.concatenate([t] * (VR_K // 8), axis=0)
            lanes.append(jnp.exp2(a + t))
        p = jnp.concatenate([jnp.exp2(s), jnp.concatenate(lanes, axis=1)], axis=0)
        return jnp.concatenate(
            [_rev8(p[t0:t0 + CK]) for t0 in range(0, SC, CK)], axis=0)

    def q_raw(blk):
        r0 = pl.multiple_of(blk * TQ, TQ)
        xb = x_ref[pl.ds(r0, TQ), :]
        q = _dot(xb, wq_ref[...]) * QSCALE
        return q

    def q_norms(qt):
        sq = (qt * qt).astype(BF16)
        hrow = lax.broadcasted_iota(jnp.int32, (H, D), 0)
        hcol = lax.broadcasted_iota(jnp.int32, (H, D), 1)
        e = jnp.logical_and(hcol >= hrow * DH, hcol < (hrow + 1) * DH)
        return _dot(jnp.where(e, 1.0, 0.0).astype(BF16), sq)

    def q_store(qt, hs):
        m2 = jnp.max(hs) * kn_ref[0] * 1.05
        safe = m2 <= SAFE_M * SAFE_M
        flag_ref[0] = safe.astype(jnp.int32)
        mval = jnp.where(safe, -jnp.sqrt(jnp.full((KD - DH, TQ), m2, F32)), 0.0)
        srow = lax.broadcasted_iota(jnp.int32, (KD - DH, TQ), 0)
        mt = jnp.where(srow == 0, mval, 0.0)
        for h in range(H):
            qw_ref[h // 2, h % 2] = jnp.concatenate(
                [qt[h * DH:(h + 1) * DH, :], mt], axis=0).astype(BF16)
        m_ref[0] = jnp.min(mt.astype(BF16).astype(F32))
        qb_ref[...] = qt.astype(BF16).astype(F32).reshape(NP, 2 * DH, TQ)

    def q_carry():
        carry_ref[...] = probs(0, 0, 0, 5, q_bcast(0, 0))

    def q_finish(qt):
        q_store(qt, q_norms(qt))
        q_carry()

    @pl.when(step == 0)
    def _init():
        early[1].start()
        early[2].start()
        x_copy(0).start()
        early[0].start()
        for c in range(1, NBLK):
            x_copy(c).start()
        wt_ref[...] = jnp.zeros_like(wt_ref)
        for i in range(NZ):
            z_ref[i] = 0
        early[1].wait()
        early[2].wait()
        wt_ref[0:DH, :] = wkt_ref[...].astype(F32)
        wt_ref[64:64 + DH, :] = wvt_ref[...].astype(F32)
        wall = wt_ref[...].T.astype(BF16)
        lane = lax.broadcasted_iota(jnp.int32, (TQ, 128), 1)
        vrow = lax.broadcasted_iota(jnp.int32, (VR, CK), 0)
        ke_fill = jnp.where(lane == DH, 1.0, 0.0)

        def kv(c, kn):
            rows = slice(c * TQ, (c + 1) * TQ)
            r = _dot(x_ref[rows, :], wall)
            r = r.astype(BF16).astype(F32)
            ke_ref[rows, :] = jnp.where(lane < DH, r, ke_fill).astype(BF16)
            for u in range(TQ // SC):
                sc = c * (TQ // SC) + u
                rv = r[u * SC + MR_K:(u + 1) * SC, :]
                for d in range(DH):
                    kb_ref[d, sc * VR_K:(sc + 1) * VR_K, :] = jnp.broadcast_to(
                        rv[:, d:d + 1], (VR_K, 128))
            for t in range(TQ // CK):
                rt = _rev8(r[t * CK:(t + 1) * CK, :]).T
                col = c * TQ + t * CK
                vt_ref[:, col:col + CK] = jnp.where(
                    vrow < DH, rt[64:64 + VR, :], jnp.where(vrow == DH, 1.0, 0.0))
                kt = rt[0:DH, :]
                n2 = jnp.sum(kt * kt, axis=0, keepdims=True)
                kn = n2 if kn is None else jnp.maximum(kn, n2)
            return kn

        x_copy(0).wait()
        early[0].wait()
        kn = kv(0, None)
        qt_ref[...] = q_raw(0)
        for c in range(1, NBLK):
            x_copy(c).wait()
        for cp in late:
            cp.start()
        for c in range(1, NBLK):
            kn = kv(c, kn)
        kn_ref[0] = jnp.max(kn)
        q_finish(qt_ref[...].T)

    def finish(acc):
        return acc[0:DH, :] * (1.0 / acc[DH:DH + 1, :])

    @pl.when(flag_ref[0] == 1)
    def _fast():
        def body(i, carry):
            j0 = i * UNROLL
            pend = carry_ref[...]
            acc = None
            n = UNROLL * 2 * NSC
            for g in range(n):
                gq = g + 1
                if gq < n:
                    jq, pq = j0 + gq // (2 * NSC), (gq // NSC) % 2
                    if gq % NSC == 0 or g == 0:
                        qbs = q_bcast(jq, pq)
                    nxt = probs(jq, pq, gq % NSC, g, qbs)
                else:
                    jq = jnp.minimum(j0 + UNROLL, NP - 1)
                    nxt = probs(jq, 0, 0, g, q_bcast(jq, 0))
                c = g % NSC
                o = _dot(vt_ref[:, c * SC:(c + 1) * SC], pend)
                acc = o if c == 0 else acc + o
                if c == NSC - 1:
                    par = (g // NSC) % 2
                    ot_ref[j0 + g // (2 * NSC), par * DH:(par + 1) * DH, :] = finish(acc)
                pend = nxt
            carry_ref[...] = pend
            return carry

        lax.fori_loop(0, NP // UNROLL, body, 0)

    @pl.when(flag_ref[0] != 1)
    def _slow():
        def head(j, par, s_ref):
            k_ref = ke_ref
            qw = qw_ref[j, par]
            m = None
            for c in range(NCK):
                s = _dot(k_ref[c * CK:(c + 1) * CK, 0:KD], qw)
                s_ref[c * CK:(c + 1) * CK, :] = s
                mc = jnp.max(s, axis=0, keepdims=True)
                m = mc if m is None else jnp.maximum(m, mc)
            acc = None
            for c in range(NCK):
                p = _rev8(jnp.exp2(s_ref[c * CK:(c + 1) * CK, :] - m))
                o = _dot(vt_ref[:, c * CK:(c + 1) * CK], p)
                acc = o if acc is None else acc + o
            ot_ref[j, par * DH:(par + 1) * DH, :] = finish(acc)

        def scoped(s_ref):
            def body(j, carry):
                head(j, 0, s_ref)
                head(j, 1, s_ref)
                return carry
            lax.fori_loop(0, NP, body, 0)

        pl.run_scoped(scoped, pltpu.VMEM((S, TQ), F32))

    @pl.when(step == 0)
    def _wait_late():
        for cp in late:
            cp.wait()

    @pl.when(step < NBLK - 1)
    def _next_q():
        qt_ref[...] = q_raw(step + 1)

    r0 = pl.multiple_of(step * TQ, TQ)
    xb = x_ref[pl.ds(r0, TQ), :]

    def hidden(fc):
        gt = _dot(xb, wg_ref[:, fc * FC:(fc + 1) * FC])
        up = _dot(xb, wu_ref[:, fc * FC:(fc + 1) * FC])
        return (jnp.maximum(gt, 0.0) * up).astype(BF16)

    nfc = F // FC
    h_prev = hidden(0)
    qt = qt_ref[...].T
    hs = q_norms(qt)
    b = None
    a = None
    for fc in range(nfc):
        if fc + 1 < nfc:
            h_next = hidden(fc + 1)
        else:
            q_carry()
            ot = ot_ref[...].reshape(D, TQ)
            a = _dot(ot.T.astype(BF16), wo_ref[...])
        if fc == 0:
            q_store(qt, hs)
        bb = _dot(h_prev, wd_ref[fc * FC:(fc + 1) * FC, :])
        b = bb if b is None else b + bb
        h_prev = h_next
    logit = jnp.sum(xb.astype(F32) * gw_ref[...].astype(F32).reshape(1, D),
                    axis=1, keepdims=True)
    g = 1.0 / (1.0 + jnp.exp(-logit))
    o_ref[0] = (g * a + (1.0 - g) * b).astype(o_ref.dtype)


@jax.jit
def pallas_gated_mix__grouped_kv_mqa__glu_gated_reglu__prompt_kernel(
    A_x: jax.Array,
    A_wq: jax.Array,
    A_wk: jax.Array,
    A_wv: jax.Array,
    A_wo: jax.Array,
    B_x: jax.Array,
    B_W_gate: jax.Array,
    B_W_up: jax.Array,
    B_W_down: jax.Array,
    gate_w: jax.Array,
):
    x = A_x.reshape(S, D)
    gw = gate_w
    hbm = pl.BlockSpec(memory_space=pl.ANY)

    return pl.pallas_call(
        _kernel,
        grid=(NBLK,),
        in_specs=[hbm] * 9,
        out_specs=pl.BlockSpec((1, TQ, D), lambda i: (0, i, 0)),
        out_shape=jax.ShapeDtypeStruct((1, S, D), BF16),
        scratch_shapes=[
            pltpu.VMEM((S, D), BF16),
            pltpu.VMEM((D, D), BF16),
            pltpu.VMEM((DH, D), BF16),
            pltpu.VMEM((DH, D), BF16),
            pltpu.VMEM((D, D), BF16),
            pltpu.VMEM((D, F), BF16),
            pltpu.VMEM((D, F), BF16),
            pltpu.VMEM((F, D), BF16),
            pltpu.VMEM((D,), BF16),
            pltpu.VMEM((S, 128), BF16),
            pltpu.VMEM((VR, S), F32),
            pltpu.VMEM((NP, 2, KD, TQ), BF16),
            pltpu.VMEM((SC, TQ), F32),
            pltpu.VMEM((NP, 2 * DH, TQ), F32),
            pltpu.VMEM((128, D), F32),
            pltpu.VMEM((TQ, D), F32),
            pltpu.VMEM((DH, NSC * VR_K, 128), F32),
            pltpu.VMEM((NP, 2 * DH, TQ), F32),
            pltpu.SMEM((1,), F32),
            pltpu.SMEM((1,), F32),
            pltpu.SMEM((1,), jnp.int32),
            pltpu.SMEM((NZ,), jnp.int32),
            pltpu.SemaphoreType.DMA((NBLK + 8,)),
        ],
        compiler_params=pltpu.CompilerParams(
            dimension_semantics=("arbitrary",),
            vmem_limit_bytes=100 * 1024 * 1024,
        ),
    )(x, A_wq, A_wk.T, A_wv.T, A_wo, B_W_gate, B_W_up, B_W_down, gw)
```

```python
import jax
import jax.numpy as jnp
from jax import lax
from jax.experimental import pallas as pl
from jax.experimental.pallas import tpu as pltpu

S = 2048
D = 640
H = 32
DH = 20
F = 1536
TQ = 512
NBLK = S // TQ
CK = 128
NCK = S // CK
SC = 256
NSC = S // SC
VR_K = 16
MR_K = SC - VR_K
GL = 256
NP = H // 2
UNROLL = 4
KD = 32
VR = 24
FC = 512
SL = 256
NZ = 64
LOG2E = 1.4426950408889634
QSCALE = (DH ** -0.5) * LOG2E
SAFE_M = 16.0

F32 = jnp.float32
BF16 = jnp.bfloat16


def _dot(a, b):
    return jnp.dot(a, b, preferred_element_type=F32)


def _rev8(p):
    n = p.shape[0] // 8
    return jnp.concatenate([p[8 * (n - 1 - t):8 * (n - t)] for t in range(n)], axis=0)


def _kernel(x_hbm, wq_hbm, wkt_hbm, wvt_hbm, wo_hbm, wg_hbm, wu_hbm, wd_hbm, gw_hbm,
            o_ref,
            x_ref, wq_ref, wkt_ref, wvt_ref, wo_ref, wg_ref, wu_ref, wd_ref, gw_ref,
            k_ref, vt_ref, qw_ref, carry_ref, ot_ref, wt_ref, q_ref,
            kb_ref, qf_ref, kn_ref, m_ref, flag_ref, z_ref, sems):
    step = pl.program_id(0)

    def x_copy(c):
        return pltpu.make_async_copy(x_hbm.at[pl.ds(c * TQ, TQ)],
                                     x_ref.at[pl.ds(c * TQ, TQ)], sems.at[c])

    early = [pltpu.make_async_copy(wq_hbm, wq_ref, sems.at[NBLK]),
             pltpu.make_async_copy(wkt_hbm, wkt_ref, sems.at[NBLK + 1]),
             pltpu.make_async_copy(wvt_hbm, wvt_ref, sems.at[NBLK + 2])]
    late = [pltpu.make_async_copy(wo_hbm, wo_ref, sems.at[NBLK + 3]),
            pltpu.make_async_copy(wg_hbm, wg_ref, sems.at[NBLK + 4]),
            pltpu.make_async_copy(wu_hbm, wu_ref, sems.at[NBLK + 5]),
            pltpu.make_async_copy(wd_hbm, wd_ref, sems.at[NBLK + 6]),
            pltpu.make_async_copy(gw_hbm, gw_ref, sems.at[NBLK + 7])]

    def q_bcast(j, par):
        return [jnp.broadcast_to(qf_ref[j, par * DH + d:par * DH + d + 1, :], (8, TQ))
                for d in range(DH)]

    def probs(j, par, c, g, qbs):
        s = _dot(k_ref[c * SC:c * SC + MR_K, 0:KD], qw_ref[j + z_ref[g % NZ], par])
        lanes = []
        for ll in range(TQ // GL):
            zi = z_ref[(g * (TQ // GL) + ll + 7) % NZ]
            a = jnp.full((VR_K, GL), m_ref[0], F32)
            for d in range(DH):
                kb = kb_ref[d + zi, c * VR_K:(c + 1) * VR_K, :]
                kb = jnp.concatenate([kb] * (GL // 128), axis=1)
                qb = qbs[d][:, ll * GL:(ll + 1) * GL]
                qb = jnp.concatenate([qb] * (VR_K // 8), axis=0)
                a = a + kb * qb
            parts = [a[rr * 8:(rr + 1) * 8, lq * 128:(lq + 1) * 128]
                     for rr in range(VR_K // 8) for lq in range(GL // 128)]
            t = parts[0]
            for part in parts[1:]:
                t = t + part
            t = t * 0.0
            t = jnp.concatenate([t] * (GL // 128), axis=1)
            t = jnp.concatenate([t] * (VR_K // 8), axis=0)
            lanes.append(jnp.exp2(a + t))
        p = jnp.concatenate([jnp.exp2(s), jnp.concatenate(lanes, axis=1)], axis=0)
        return jnp.concatenate(
            [_rev8(p[t0:t0 + CK]) for t0 in range(0, SC, CK)], axis=0)

    def q_raw(blk):
        r0 = pl.multiple_of(blk * TQ, TQ)
        return _dot(x_ref[pl.ds(r0, TQ), :], wq_ref[...]) * QSCALE

    def q_norms(qt):
        sq = (qt * qt).astype(BF16)
        hrow = lax.broadcasted_iota(jnp.int32, (H, D), 0)
        hcol = lax.broadcasted_iota(jnp.int32, (H, D), 1)
        e = jnp.logical_and(hcol >= hrow * DH, hcol < (hrow + 1) * DH)
        return _dot(jnp.where(e, 1.0, 0.0).astype(BF16), sq)

    def q_store(qt, hs):
        m2 = jnp.max(hs) * kn_ref[0] * 1.05
        safe = m2 <= SAFE_M * SAFE_M
        flag_ref[0] = safe.astype(jnp.int32)
        mval = jnp.where(safe, -jnp.sqrt(jnp.full((KD - DH, TQ), m2, F32)), 0.0)
        srow = lax.broadcasted_iota(jnp.int32, (KD - DH, TQ), 0)
        mt = jnp.where(srow == 0, mval, 0.0)
        for h in range(H):
            qw_ref[h // 2, h % 2] = jnp.concatenate(
                [qt[h * DH:(h + 1) * DH, :], mt], axis=0).astype(BF16)
        m_ref[0] = jnp.min(mt.astype(BF16).astype(F32))
        qf_ref[...] = qt.astype(BF16).astype(F32).reshape(NP, 2 * DH, TQ)

    def q_carry():
        carry_ref[...] = probs(0, 0, 0, 5, q_bcast(0, 0))

    @pl.when(step == 0)
    def _init():
        early[1].start()
        early[2].start()
        x_copy(0).start()
        early[0].start()
        for c in range(1, NBLK):
            x_copy(c).start()
        wt_ref[...] = jnp.zeros_like(wt_ref)
        for i in range(NZ):
            z_ref[i] = 0
        early[1].wait()
        early[2].wait()
        wt_ref[0:DH, :] = wkt_ref[...].astype(F32)
        wt_ref[64:64 + DH, :] = wvt_ref[...].astype(F32)
        wall = wt_ref[...].T.astype(BF16)
        lane = lax.broadcasted_iota(jnp.int32, (TQ, 128), 1)
        vrow = lax.broadcasted_iota(jnp.int32, (VR, CK), 0)
        k_fill = jnp.where(lane == DH, 1.0, 0.0)

        def kv(c, kn):
            rows = slice(c * TQ, (c + 1) * TQ)
            r = _dot(x_ref[rows, :], wall)
            r = r.astype(BF16).astype(F32)
            k_ref[rows, :] = jnp.where(lane < DH, r, k_fill).astype(BF16)
            for u in range(TQ // SC):
                sc = c * (TQ // SC) + u
                rv = r[u * SC + MR_K:(u + 1) * SC, :]
                for d in range(DH):
                    kb_ref[d, sc * VR_K:(sc + 1) * VR_K, :] = jnp.broadcast_to(
                        rv[:, d:d + 1], (VR_K, 128))
            for t in range(TQ // CK):
                rt = _rev8(r[t * CK:(t + 1) * CK, :]).T
                col = c * TQ + t * CK
                vt_ref[:, col:col + CK] = jnp.where(
                    vrow < DH, rt[64:64 + VR, :], jnp.where(vrow == DH, 1.0, 0.0))
                kt = rt[0:DH, :]
                n2 = jnp.sum(kt * kt, axis=0, keepdims=True)
                kn = n2 if kn is None else jnp.maximum(kn, n2)
            return kn

        x_copy(0).wait()
        early[0].wait()
        kn = kv(0, None)
        q_ref[...] = q_raw(0)
        for c in range(1, NBLK):
            x_copy(c).wait()
        for cp in late:
            cp.start()
        for c in range(1, NBLK):
            kn = kv(c, kn)
        kn_ref[0] = jnp.max(kn)
        qt0 = q_ref[...].T
        q_store(qt0, q_norms(qt0))
        q_carry()

    def finish(acc):
        return acc[0:DH, :] * (1.0 / acc[DH:DH + 1, :])

    @pl.when(flag_ref[0] == 1)
    def _fast():
        def body(i, carry):
            j0 = i * UNROLL
            pend = carry_ref[...]
            acc = None
            n = UNROLL * 2 * NSC
            for g in range(n):
                gq = g + 1
                if gq < n:
                    jq, pq = j0 + gq // (2 * NSC), (gq // NSC) % 2
                    if gq % NSC == 0 or g == 0:
                        qbs = q_bcast(jq, pq)
                    nxt = probs(jq, pq, gq % NSC, g, qbs)
                else:
                    jq = jnp.minimum(j0 + UNROLL, NP - 1)
                    nxt = probs(jq, 0, 0, g, q_bcast(jq, 0))
                c = g % NSC
                o = _dot(vt_ref[:, c * SC:(c + 1) * SC], pend)
                acc = o if c == 0 else acc + o
                if c == NSC - 1:
                    par = (g // NSC) % 2
                    ot_ref[j0 + g // (2 * NSC), par * DH:(par + 1) * DH, :] = finish(acc)
                pend = nxt
            carry_ref[...] = pend
            return carry

        lax.fori_loop(0, NP // UNROLL, body, 0)

    @pl.when(flag_ref[0] != 1)
    def _slow():
        def head(j, par, s_ref):
            qw = qw_ref[j, par]
            m = None
            for c in range(NCK):
                s = _dot(k_ref[c * CK:(c + 1) * CK, 0:KD], qw)
                s_ref[c * CK:(c + 1) * CK, :] = s
                mc = jnp.max(s, axis=0, keepdims=True)
                m = mc if m is None else jnp.maximum(m, mc)
            acc = None
            for c in range(NCK):
                p = _rev8(jnp.exp2(s_ref[c * CK:(c + 1) * CK, :] - m))
                o = _dot(vt_ref[:, c * CK:(c + 1) * CK], p)
                acc = o if acc is None else acc + o
            ot_ref[j, par * DH:(par + 1) * DH, :] = finish(acc)

        def scoped(s_ref):
            def body(j, carry):
                head(j, 0, s_ref)
                head(j, 1, s_ref)
                return carry
            lax.fori_loop(0, NP, body, 0)

        pl.run_scoped(scoped, pltpu.VMEM((S, TQ), F32))

    @pl.when(step == 0)
    def _wait_late():
        for cp in late:
            cp.wait()

    @pl.when(step < NBLK - 1)
    def _next_q():
        q_ref[...] = q_raw(step + 1)

    r0 = pl.multiple_of(step * TQ, TQ)
    xb = x_ref[pl.ds(r0, TQ), :]
    nsl = TQ // SL
    nfc = F // FC

    def hidden(fc, sl):
        xs = xb[sl * SL:(sl + 1) * SL, :]
        gt = _dot(xs, wg_ref[:, fc * FC:(fc + 1) * FC])
        up = _dot(xs, wu_ref[:, fc * FC:(fc + 1) * FC])
        return (jnp.maximum(gt, 0.0) * up).astype(BF16)

    h_prev = [hidden(0, sl) for sl in range(nsl)]
    qt = q_ref[...].T
    hs = q_norms(qt)
    b = [None] * nsl
    a = [None] * nsl
    o_nat = None
    for fc in range(nfc):
        h_next = [None] * nsl
        for sl in range(nsl):
            if fc + 1 < nfc:
                h_next[sl] = hidden(fc + 1, sl)
            else:
                if sl == 0:
                    q_carry()
                    o_nat = ot_ref[...].reshape(D, TQ).T.astype(BF16)
                a[sl] = _dot(o_nat[sl * SL:(sl + 1) * SL, :], wo_ref[...])
            if fc == 0 and sl == 0:
                q_store(qt, hs)
            bb = _dot(h_prev[sl], wd_ref[fc * FC:(fc + 1) * FC, :])
            b[sl] = bb if b[sl] is None else b[sl] + bb
        h_prev = h_next
    a = jnp.concatenate(a, axis=0)
    b = jnp.concatenate(b, axis=0)
    logit = jnp.sum(xb.astype(F32) * gw_ref[...].astype(F32).reshape(1, D),
                    axis=1, keepdims=True)
    g = 1.0 / (1.0 + jnp.exp(-logit))
    o_ref[0] = (g * a + (1.0 - g) * b).astype(o_ref.dtype)


@jax.jit
def pallas_gated_mix__grouped_kv_mqa__glu_gated_reglu__prompt_kernel(
    A_x: jax.Array,
    A_wq: jax.Array,
    A_wk: jax.Array,
    A_wv: jax.Array,
    A_wo: jax.Array,
    B_x: jax.Array,
    B_W_gate: jax.Array,
    B_W_up: jax.Array,
    B_W_down: jax.Array,
    gate_w: jax.Array,
):
    del B_x
    hbm = pl.BlockSpec(memory_space=pl.ANY)

    return pl.pallas_call(
        _kernel,
        grid=(NBLK,),
        in_specs=[hbm] * 9,
        out_specs=pl.BlockSpec((1, TQ, D), lambda i: (0, i, 0)),
        out_shape=jax.ShapeDtypeStruct((1, S, D), BF16),
        scratch_shapes=[
            pltpu.VMEM((S, D), BF16),
            pltpu.VMEM((D, D), BF16),
            pltpu.VMEM((DH, D), BF16),
            pltpu.VMEM((DH, D), BF16),
            pltpu.VMEM((D, D), BF16),
            pltpu.VMEM((D, F), BF16),
            pltpu.VMEM((D, F), BF16),
            pltpu.VMEM((F, D), BF16),
            pltpu.VMEM((D,), BF16),
            pltpu.VMEM((S, 128), BF16),
            pltpu.VMEM((VR, S), F32),
            pltpu.VMEM((NP, 2, KD, TQ), BF16),
            pltpu.VMEM((SC, TQ), F32),
            pltpu.VMEM((NP, 2 * DH, TQ), F32),
            pltpu.VMEM((128, D), F32),
            pltpu.VMEM((TQ, D), F32),
            pltpu.VMEM((DH, NSC * VR_K, 128), F32),
            pltpu.VMEM((NP, 2 * DH, TQ), F32),
            pltpu.SMEM((1,), F32),
            pltpu.SMEM((1,), F32),
            pltpu.SMEM((1,), jnp.int32),
            pltpu.SMEM((NZ,), jnp.int32),
            pltpu.SemaphoreType.DMA((NBLK + 8,)),
        ],
        compiler_params=pltpu.CompilerParams(
            dimension_semantics=("arbitrary",),
            vmem_limit_bytes=100 * 1024 * 1024,
        ),
    )(A_x.reshape(S, D), A_wq, A_wk.T, A_wv.T, A_wo, B_W_gate, B_W_up, B_W_down, gate_w)
```

```python
import jax
import jax.numpy as jnp
from jax import lax
from jax.experimental import pallas as pl
from jax.experimental.pallas import tpu as pltpu

S = 2048
D = 640
H = 32
DH = 20
F = 1536
TQ = 512
NBLK = S // TQ
CK = 128
NCK = S // CK
SC = 256
NSC = S // SC
VR_K = 16
MR_K = SC - VR_K
GL = 256
NP = H // 2
UNROLL = 4
KD = 32
VR = 24
FC = 512
SL = 256
NZ = 64
LOG2E = 1.4426950408889634
QSCALE = (DH ** -0.5) * LOG2E
SAFE_M = 16.0

F32 = jnp.float32
BF16 = jnp.bfloat16


def _dot(a, b):
    return jnp.dot(a, b, preferred_element_type=F32)


def _pk(x):
    return pltpu.bitcast(x, jnp.uint32)


def _unpk(x):
    return pltpu.bitcast(x, BF16)


def _rev8(p):
    n = p.shape[0] // 8
    return jnp.concatenate([p[8 * (n - 1 - t):8 * (n - t)] for t in range(n)], axis=0)


def _kernel(x_hbm, wq_hbm, wkt_hbm, wvt_hbm, wo_hbm, wg_hbm, wu_hbm, wd_hbm, gw_hbm,
            o_ref,
            x_ref, wq_ref, wkt_ref, wvt_ref, wo_ref, wg_ref, wu_ref, wd_ref, gw_ref,
            k_ref, vt_ref, qw_ref, carry_ref, ot_ref, wt_ref, q_ref,
            kb_ref, qf_ref, kn_ref, m_ref, flag_ref, z_ref, sems):
    step = pl.program_id(0)

    def x_copy(c):
        return pltpu.make_async_copy(x_hbm.at[pl.ds(c * TQ, TQ)],
                                     x_ref.at[pl.ds(c * TQ, TQ)], sems.at[c])

    early = [pltpu.make_async_copy(wq_hbm, wq_ref, sems.at[NBLK]),
             pltpu.make_async_copy(wkt_hbm, wkt_ref, sems.at[NBLK + 1]),
             pltpu.make_async_copy(wvt_hbm, wvt_ref, sems.at[NBLK + 2])]
    late = [pltpu.make_async_copy(wo_hbm, wo_ref, sems.at[NBLK + 3]),
            pltpu.make_async_copy(wg_hbm, wg_ref, sems.at[NBLK + 4]),
            pltpu.make_async_copy(wu_hbm, wu_ref, sems.at[NBLK + 5]),
            pltpu.make_async_copy(wd_hbm, wd_ref, sems.at[NBLK + 6]),
            pltpu.make_async_copy(gw_hbm, gw_ref, sems.at[NBLK + 7])]

    def k_rows(r0, n):
        return _unpk(k_ref[r0 // 2:(r0 + n) // 2, :])[:, 0:KD]

    def q_bcast(j, par):
        return [jnp.broadcast_to(qf_ref[j, par * DH + d:par * DH + d + 1, :], (8, TQ))
                for d in range(DH)]

    def probs(j, par, c, g, qbs):
        s = _dot(k_rows(c * SC, MR_K), _unpk(qw_ref[j + z_ref[g % NZ], par]))
        lanes = []
        for ll in range(TQ // GL):
            zi = z_ref[(g * (TQ // GL) + ll + 7) % NZ]
            a = jnp.full((VR_K, GL), m_ref[0], F32)
            for d in range(DH):
                kb = kb_ref[d + zi, c * VR_K:(c + 1) * VR_K, :]
                kb = jnp.concatenate([kb] * (GL // 128), axis=1)
                qb = qbs[d][:, ll * GL:(ll + 1) * GL]
                qb = jnp.concatenate([qb] * (VR_K // 8), axis=0)
                a = a + kb * qb
            parts = [a[rr * 8:(rr + 1) * 8, lq * 128:(lq + 1) * 128]
                     for rr in range(VR_K // 8) for lq in range(GL // 128)]
            t = parts[0]
            for part in parts[1:]:
                t = t + part
            t = t * 0.0
            t = jnp.concatenate([t] * (GL // 128), axis=1)
            t = jnp.concatenate([t] * (VR_K // 8), axis=0)
            lanes.append(jnp.exp2(a + t))
        p = jnp.concatenate([jnp.exp2(s), jnp.concatenate(lanes, axis=1)], axis=0)
        return jnp.concatenate(
            [_rev8(p[t0:t0 + CK]) for t0 in range(0, SC, CK)], axis=0)

    def q_raw(blk):
        r0 = pl.multiple_of(blk * TQ, TQ)
        return _dot(x_ref[pl.ds(r0, TQ), :], wq_ref[...]) * QSCALE

    def q_norms(qt):
        sq = (qt * qt).astype(BF16)
        hrow = lax.broadcasted_iota(jnp.int32, (H, D), 0)
        hcol = lax.broadcasted_iota(jnp.int32, (H, D), 1)
        e = jnp.logical_and(hcol >= hrow * DH, hcol < (hrow + 1) * DH)
        return _dot(jnp.where(e, 1.0, 0.0).astype(BF16), sq)

    def q_store(qt, hs):
        m2 = jnp.max(hs) * kn_ref[0] * 1.05
        safe = m2 <= SAFE_M * SAFE_M
        flag_ref[0] = safe.astype(jnp.int32)
        mval = jnp.where(safe, -jnp.sqrt(jnp.full((KD - DH, TQ), m2, F32)), 0.0)
        srow = lax.broadcasted_iota(jnp.int32, (KD - DH, TQ), 0)
        mt = jnp.where(srow == 0, mval, 0.0)
        for h in range(H):
            qw_ref[h // 2, h % 2] = _pk(jnp.concatenate(
                [qt[h * DH:(h + 1) * DH, :], mt], axis=0).astype(BF16))
        m_ref[0] = jnp.min(mt.astype(BF16).astype(F32))
        qf_ref[...] = qt.astype(BF16).astype(F32).reshape(NP, 2 * DH, TQ)

    def q_carry():
        carry_ref[...] = probs(0, 0, 0, 5, q_bcast(0, 0))

    @pl.when(step == 0)
    def _init():
        early[1].start()
        early[2].start()
        x_copy(0).start()
        early[0].start()
        for c in range(1, NBLK):
            x_copy(c).start()
        wt_ref[...] = jnp.zeros_like(wt_ref)
        for i in range(NZ):
            z_ref[i] = 0
        early[1].wait()
        early[2].wait()
        wt_ref[0:DH, :] = wkt_ref[...].astype(F32)
        wt_ref[64:64 + DH, :] = wvt_ref[...].astype(F32)
        wall = wt_ref[...].T.astype(BF16)
        lane = lax.broadcasted_iota(jnp.int32, (TQ, 128), 1)
        vrow = lax.broadcasted_iota(jnp.int32, (VR, CK), 0)
        k_fill = jnp.where(lane == DH, 1.0, 0.0)

        def kv(c, kn):
            rows = slice(c * TQ, (c + 1) * TQ)
            r = _dot(x_ref[rows, :], wall)
            r = r.astype(BF16).astype(F32)
            k_ref[c * TQ // 2:(c + 1) * TQ // 2, :] = _pk(
                jnp.where(lane < DH, r, k_fill).astype(BF16))
            for u in range(TQ // SC):
                sc = c * (TQ // SC) + u
                rv = r[u * SC + MR_K:(u + 1) * SC, :]
                for d in range(DH):
                    kb_ref[d, sc * VR_K:(sc + 1) * VR_K, :] = jnp.broadcast_to(
                        rv[:, d:d + 1], (VR_K, 128))
            for t in range(TQ // CK):
                rt = _rev8(r[t * CK:(t + 1) * CK, :]).T
                col = c * TQ + t * CK
                vt_ref[:, col:col + CK] = jnp.where(
                    vrow < DH, rt[64:64 + VR, :], jnp.where(vrow == DH, 1.0, 0.0))
                kt = rt[0:DH, :]
                n2 = jnp.sum(kt * kt, axis=0, keepdims=True)
                kn = n2 if kn is None else jnp.maximum(kn, n2)
            return kn

        x_copy(0).wait()
        early[0].wait()
        kn = kv(0, None)
        q_ref[...] = q_raw(0)
        for c in range(1, NBLK):
            x_copy(c).wait()
        for cp in late:
            cp.start()
        for c in range(1, NBLK):
            kn = kv(c, kn)
        kn_ref[0] = jnp.max(kn)
        qt0 = q_ref[...].T
        q_store(qt0, q_norms(qt0))
        q_carry()

    def finish(acc):
        return acc[0:DH, :] * (1.0 / acc[DH:DH + 1, :])

    @pl.when(flag_ref[0] == 1)
    def _fast():
        def body(i, carry):
            j0 = i * UNROLL
            pend = carry_ref[...]
            acc = None
            n = UNROLL * 2 * NSC
            for g in range(n):
                gq = g + 1
                if gq < n:
                    jq, pq = j0 + gq // (2 * NSC), (gq // NSC) % 2
                    if gq % NSC == 0 or g == 0:
                        qbs = q_bcast(jq, pq)
                    nxt = probs(jq, pq, gq % NSC, g, qbs)
                else:
                    jq = jnp.minimum(j0 + UNROLL, NP - 1)
                    nxt = probs(jq, 0, 0, g, q_bcast(jq, 0))
                c = g % NSC
                o = _dot(vt_ref[:, c * SC:(c + 1) * SC], pend)
                acc = o if c == 0 else acc + o
                if c == NSC - 1:
                    par = (g // NSC) % 2
                    ot_ref[j0 + g // (2 * NSC), par * DH:(par + 1) * DH, :] = finish(acc)
                pend = nxt
            carry_ref[...] = pend
            return carry

        lax.fori_loop(0, NP // UNROLL, body, 0)

    @pl.when(flag_ref[0] != 1)
    def _slow():
        def head(j, par, s_ref):
            qw = _unpk(qw_ref[j, par])
            m = None
            for c in range(NCK):
                s = _dot(k_rows(c * CK, CK), qw)
                s_ref[c * CK:(c + 1) * CK, :] = s
                mc = jnp.max(s, axis=0, keepdims=True)
                m = mc if m is None else jnp.maximum(m, mc)
            acc = None
            for c in range(NCK):
                p = _rev8(jnp.exp2(s_ref[c * CK:(c + 1) * CK, :] - m))
                o = _dot(vt_ref[:, c * CK:(c + 1) * CK], p)
                acc = o if acc is None else acc + o
            ot_ref[j, par * DH:(par + 1) * DH, :] = finish(acc)

        def scoped(s_ref):
            def body(j, carry):
                head(j, 0, s_ref)
                head(j, 1, s_ref)
                return carry
            lax.fori_loop(0, NP, body, 0)

        pl.run_scoped(scoped, pltpu.VMEM((S, TQ), F32))

    @pl.when(step == 0)
    def _wait_late():
        for cp in late:
            cp.wait()

    @pl.when(step < NBLK - 1)
    def _next_q():
        q_ref[...] = q_raw(step + 1)

    r0 = pl.multiple_of(step * TQ, TQ)
    xb = x_ref[pl.ds(r0, TQ), :]
    nsl = TQ // SL
    nfc = F // FC

    def hidden(fc, sl):
        xs = xb[sl * SL:(sl + 1) * SL, :]
        gt = _dot(xs, wg_ref[:, fc * FC:(fc + 1) * FC])
        up = _dot(xs, wu_ref[:, fc * FC:(fc + 1) * FC])
        return (jnp.maximum(gt, 0.0) * up).astype(BF16)

    h_prev = [hidden(0, sl) for sl in range(nsl)]
    qt = q_ref[...].T
    hs = q_norms(qt)
    b = [None] * nsl
    a = [None] * nsl
    o_nat = None
    for fc in range(nfc):
        h_next = [None] * nsl
        for sl in range(nsl):
            if fc + 1 < nfc:
                h_next[sl] = hidden(fc + 1, sl)
            else:
                if sl == 0:
                    q_carry()
                    o_nat = ot_ref[...].reshape(D, TQ).T.astype(BF16)
                a[sl] = _dot(o_nat[sl * SL:(sl + 1) * SL, :], wo_ref[...])
            if fc == 0 and sl == 0:
                q_store(qt, hs)
            bb = _dot(h_prev[sl], wd_ref[fc * FC:(fc + 1) * FC, :])
            b[sl] = bb if b[sl] is None else b[sl] + bb
        h_prev = h_next
    a = jnp.concatenate(a, axis=0)
    b = jnp.concatenate(b, axis=0)
    logit = jnp.sum(xb.astype(F32) * gw_ref[...].astype(F32).reshape(1, D),
                    axis=1, keepdims=True)
    g = 1.0 / (1.0 + jnp.exp(-logit))
    o_ref[0] = (g * a + (1.0 - g) * b).astype(o_ref.dtype)


@jax.jit
def pallas_gated_mix__grouped_kv_mqa__glu_gated_reglu__prompt_kernel(
    A_x: jax.Array,
    A_wq: jax.Array,
    A_wk: jax.Array,
    A_wv: jax.Array,
    A_wo: jax.Array,
    B_x: jax.Array,
    B_W_gate: jax.Array,
    B_W_up: jax.Array,
    B_W_down: jax.Array,
    gate_w: jax.Array,
):
    del B_x
    hbm = pl.BlockSpec(memory_space=pl.ANY)

    return pl.pallas_call(
        _kernel,
        grid=(NBLK,),
        in_specs=[hbm] * 9,
        out_specs=pl.BlockSpec((1, TQ, D), lambda i: (0, i, 0)),
        out_shape=jax.ShapeDtypeStruct((1, S, D), BF16),
        scratch_shapes=[
            pltpu.VMEM((S, D), BF16),
            pltpu.VMEM((D, D), BF16),
            pltpu.VMEM((DH, D), BF16),
            pltpu.VMEM((DH, D), BF16),
            pltpu.VMEM((D, D), BF16),
            pltpu.VMEM((D, F), BF16),
            pltpu.VMEM((D, F), BF16),
            pltpu.VMEM((F, D), BF16),
            pltpu.VMEM((D,), BF16),
            pltpu.VMEM((S // 2, 128), jnp.uint32),
            pltpu.VMEM((VR, S), F32),
            pltpu.VMEM((NP, 2, KD // 2, TQ), jnp.uint32),
            pltpu.VMEM((SC, TQ), F32),
            pltpu.VMEM((NP, 2 * DH, TQ), F32),
            pltpu.VMEM((128, D), F32),
            pltpu.VMEM((TQ, D), F32),
            pltpu.VMEM((DH, NSC * VR_K, 128), F32),
            pltpu.VMEM((NP, 2 * DH, TQ), F32),
            pltpu.SMEM((1,), F32),
            pltpu.SMEM((1,), F32),
            pltpu.SMEM((1,), jnp.int32),
            pltpu.SMEM((NZ,), jnp.int32),
            pltpu.SemaphoreType.DMA((NBLK + 8,)),
        ],
        compiler_params=pltpu.CompilerParams(
            dimension_semantics=("arbitrary",),
            vmem_limit_bytes=100 * 1024 * 1024,
        ),
    )(A_x.reshape(S, D), A_wq, A_wk.T, A_wv.T, A_wo, B_W_gate, B_W_up, B_W_down, gate_w)
```

```python
import jax
import jax.numpy as jnp
from jax import lax
from jax.experimental import pallas as pl
from jax.experimental.pallas import tpu as pltpu

S = 2048
D = 640
H = 32
DH = 20
F = 1536
TQ = 512
NBLK = S // TQ
CK = 128
NCK = S // CK
SC = 256
NSC = S // SC
VRS = [0] + [16] * (NSC - 1)
VOFF = [sum(VRS[:c]) for c in range(NSC)]
NVK = sum(VRS)
GR = 16
GL = 256
NP = H // 2
UNROLL = 4
KD = 32
VR = 24
FC = 512
SL = 256
NZ = 64
LOG2E = 1.4426950408889634
QSCALE = (DH ** -0.5) * LOG2E
SAFE_M = 16.0

F32 = jnp.float32
BF16 = jnp.bfloat16


def _dot(a, b):
    return jnp.dot(a, b, preferred_element_type=F32)


def _pk(x):
    return pltpu.bitcast(x, jnp.uint32)


def _unpk(x):
    return pltpu.bitcast(x, BF16)


def _rev8(p):
    n = p.shape[0] // 8
    return jnp.concatenate([p[8 * (n - 1 - t):8 * (n - t)] for t in range(n)], axis=0)


def _kernel(x_hbm, wq_hbm, wkt_hbm, wvt_hbm, wo_hbm, wg_hbm, wu_hbm, wd_hbm, gw_hbm,
            o_ref,
            x_ref, wq_ref, wkt_ref, wvt_ref, wo_ref, wg_ref, wu_ref, wd_ref, gw_ref,
            k_ref, vt_ref, qw_ref, carry_ref, ot_ref, wt_ref, q_ref,
            kb_ref, qf_ref, kn_ref, m_ref, flag_ref, z_ref, sems):
    step = pl.program_id(0)

    def x_copy(c):
        return pltpu.make_async_copy(x_hbm.at[pl.ds(c * TQ, TQ)],
                                     x_ref.at[pl.ds(c * TQ, TQ)], sems.at[c])

    early = [pltpu.make_async_copy(wq_hbm, wq_ref, sems.at[NBLK]),
             pltpu.make_async_copy(wkt_hbm, wkt_ref, sems.at[NBLK + 1]),
             pltpu.make_async_copy(wvt_hbm, wvt_ref, sems.at[NBLK + 2])]
    late = [pltpu.make_async_copy(wo_hbm, wo_ref, sems.at[NBLK + 3]),
            pltpu.make_async_copy(wg_hbm, wg_ref, sems.at[NBLK + 4]),
            pltpu.make_async_copy(wu_hbm, wu_ref, sems.at[NBLK + 5]),
            pltpu.make_async_copy(wd_hbm, wd_ref, sems.at[NBLK + 6]),
            pltpu.make_async_copy(gw_hbm, gw_ref, sems.at[NBLK + 7])]

    def k_rows(r0, n):
        return _unpk(k_ref[r0 // 2:(r0 + n) // 2, :])[:, 0:KD]

    def q_bcast(j, par):
        return [jnp.broadcast_to(qf_ref[j, par * DH + d:par * DH + d + 1, :], (8, TQ))
                for d in range(DH)]

    def probs(j, par, c, g, qbs):
        s = _dot(k_rows(c * SC, SC - VRS[c]), _unpk(qw_ref[j + z_ref[g % NZ], par]))
        vrows = []
        for gg in range(VRS[c] // GR):
            r0 = VOFF[c] + gg * GR
            lanes = []
            for ll in range(TQ // GL):
                zi = z_ref[(g * 8 + gg * (TQ // GL) + ll + 7) % NZ]
                a = jnp.full((GR, GL), m_ref[0], F32)
                for d in range(DH):
                    kb = kb_ref[d + zi, r0:r0 + GR, :]
                    kb = jnp.concatenate([kb] * (GL // 128), axis=1)
                    qb = qbs[d][:, ll * GL:(ll + 1) * GL]
                    qb = jnp.concatenate([qb] * (GR // 8), axis=0)
                    a = a + kb * qb
                parts = [a[rr * 8:(rr + 1) * 8, lq * 128:(lq + 1) * 128]
                         for rr in range(GR // 8) for lq in range(GL // 128)]
                t = parts[0]
                for part in parts[1:]:
                    t = t + part
                t = t * 0.0
                t = jnp.concatenate([t] * (GL // 128), axis=1)
                t = jnp.concatenate([t] * (GR // 8), axis=0)
                lanes.append(jnp.exp2(a + t))
            vrows.append(jnp.concatenate(lanes, axis=1))
        p = jnp.concatenate([jnp.exp2(s)] + vrows, axis=0)
        return jnp.concatenate(
            [_rev8(p[t0:t0 + CK]) for t0 in range(0, SC, CK)], axis=0)

    def q_raw(blk):
        r0 = pl.multiple_of(blk * TQ, TQ)
        return _dot(x_ref[pl.ds(r0, TQ), :], wq_ref[...]) * QSCALE

    def q_norms(qt):
        sq = (qt * qt).astype(BF16)
        hrow = lax.broadcasted_iota(jnp.int32, (H, D), 0)
        hcol = lax.broadcasted_iota(jnp.int32, (H, D), 1)
        e = jnp.logical_and(hcol >= hrow * DH, hcol < (hrow + 1) * DH)
        return _dot(jnp.where(e, 1.0, 0.0).astype(BF16), sq)

    def q_store(qt, hs):
        m2 = jnp.max(hs) * kn_ref[0] * 1.05
        safe = m2 <= SAFE_M * SAFE_M
        flag_ref[0] = safe.astype(jnp.int32)
        mval = jnp.where(safe, -jnp.sqrt(jnp.full((KD - DH, TQ), m2, F32)), 0.0)
        srow = lax.broadcasted_iota(jnp.int32, (KD - DH, TQ), 0)
        mt = jnp.where(srow == 0, mval, 0.0)
        for h in range(H):
            qw_ref[h // 2, h % 2] = _pk(jnp.concatenate(
                [qt[h * DH:(h + 1) * DH, :], mt], axis=0).astype(BF16))
        m_ref[0] = jnp.min(mt.astype(BF16).astype(F32))
        qf_ref[...] = qt.astype(BF16).astype(F32).reshape(NP, 2 * DH, TQ)

    def q_carry():
        carry_ref[...] = probs(0, 0, 0, 5, q_bcast(0, 0))

    @pl.when(step == 0)
    def _init():
        early[1].start()
        early[2].start()
        x_copy(0).start()
        early[0].start()
        for c in range(1, NBLK):
            x_copy(c).start()
        wt_ref[...] = jnp.zeros_like(wt_ref)
        for i in range(NZ):
            z_ref[i] = 0
        early[1].wait()
        early[2].wait()
        wt_ref[0:DH, :] = wkt_ref[...].astype(F32)
        wt_ref[64:64 + DH, :] = wvt_ref[...].astype(F32)
        wall = wt_ref[...].T.astype(BF16)
        lane = lax.broadcasted_iota(jnp.int32, (TQ, 128), 1)
        vrow = lax.broadcasted_iota(jnp.int32, (VR, CK), 0)
        k_fill = jnp.where(lane == DH, 1.0, 0.0)

        def kv(c, kn):
            rows = slice(c * TQ, (c + 1) * TQ)
            r = _dot(x_ref[rows, :], wall)
            r = r.astype(BF16).astype(F32)
            k_ref[c * TQ // 2:(c + 1) * TQ // 2, :] = _pk(
                jnp.where(lane < DH, r, k_fill).astype(BF16))
            for u in range(TQ // SC):
                sc = c * (TQ // SC) + u
                if VRS[sc]:
                    rv = r[(u + 1) * SC - VRS[sc]:(u + 1) * SC, :]
                    for d in range(DH):
                        kb_ref[d, VOFF[sc]:VOFF[sc] + VRS[sc], :] = jnp.broadcast_to(
                            rv[:, d:d + 1], (VRS[sc], 128))
            for t in range(TQ // CK):
                rt = _rev8(r[t * CK:(t + 1) * CK, :]).T
                col = c * TQ + t * CK
                vt_ref[:, col:col + CK] = jnp.where(
                    vrow < DH, rt[64:64 + VR, :], jnp.where(vrow == DH, 1.0, 0.0))
                kt = rt[0:DH, :]
                n2 = jnp.sum(kt * kt, axis=0, keepdims=True)
                kn = n2 if kn is None else jnp.maximum(kn, n2)
            return kn

        x_copy(0).wait()
        early[0].wait()
        kn = kv(0, None)
        q_ref[...] = q_raw(0)
        for c in range(1, NBLK):
            x_copy(c).wait()
        for cp in late:
            cp.start()
        for c in range(1, NBLK):
            kn = kv(c, kn)
        kn_ref[0] = jnp.max(kn)
        qt0 = q_ref[...].T
        q_store(qt0, q_norms(qt0))
        q_carry()

    def finish(acc):
        return acc[0:DH, :] * (1.0 / acc[DH:DH + 1, :])

    @pl.when(flag_ref[0] == 1)
    def _fast():
        def body(i, carry):
            j0 = i * UNROLL
            pend = carry_ref[...]
            acc = None
            n = UNROLL * 2 * NSC
            for g in range(n):
                gq = g + 1
                if gq < n:
                    jq, pq = j0 + gq // (2 * NSC), (gq // NSC) % 2
                    if gq % NSC == 0 or g == 0:
                        qbs = q_bcast(jq, pq)
                    nxt = probs(jq, pq, gq % NSC, g, qbs)
                else:
                    jq = jnp.minimum(j0 + UNROLL, NP - 1)
                    nxt = probs(jq, 0, 0, g, q_bcast(jq, 0))
                c = g % NSC
                o = _dot(vt_ref[:, c * SC:(c + 1) * SC], pend)
                acc = o if c == 0 else acc + o
                if c == NSC - 1:
                    par = (g // NSC) % 2
                    ot_ref[j0 + g // (2 * NSC), par * DH:(par + 1) * DH, :] = finish(acc)
                pend = nxt
            carry_ref[...] = pend
            return carry

        lax.fori_loop(0, NP // UNROLL, body, 0)

    @pl.when(flag_ref[0] != 1)
    def _slow():
        def head(j, par, s_ref):
            qw = _unpk(qw_ref[j, par])
            m = None
            for c in range(NCK):
                s = _dot(k_rows(c * CK, CK), qw)
                s_ref[c * CK:(c + 1) * CK, :] = s
                mc = jnp.max(s, axis=0, keepdims=True)
                m = mc if m is None else jnp.maximum(m, mc)
            acc = None
            for c in range(NCK):
                p = _rev8(jnp.exp2(s_ref[c * CK:(c + 1) * CK, :] - m))
                o = _dot(vt_ref[:, c * CK:(c + 1) * CK], p)
                acc = o if acc is None else acc + o
            ot_ref[j, par * DH:(par + 1) * DH, :] = finish(acc)

        def scoped(s_ref):
            def body(j, carry):
                head(j, 0, s_ref)
                head(j, 1, s_ref)
                return carry
            lax.fori_loop(0, NP, body, 0)

        pl.run_scoped(scoped, pltpu.VMEM((S, TQ), F32))

    @pl.when(step == 0)
    def _wait_late():
        for cp in late:
            cp.wait()

    @pl.when(step < NBLK - 1)
    def _next_q():
        q_ref[...] = q_raw(step + 1)

    r0 = pl.multiple_of(step * TQ, TQ)
    xb = x_ref[pl.ds(r0, TQ), :]
    nsl = TQ // SL
    nfc = F // FC

    def hidden(fc, sl):
        xs = xb[sl * SL:(sl + 1) * SL, :]
        gt = _dot(xs, wg_ref[:, fc * FC:(fc + 1) * FC])
        up = _dot(xs, wu_ref[:, fc * FC:(fc + 1) * FC])
        return (jnp.maximum(gt, 0.0) * up).astype(BF16)

    h_prev = [hidden(0, sl) for sl in range(nsl)]
    qt = q_ref[...].T
    hs = q_norms(qt)
    b = [None] * nsl
    a = [None] * nsl
    o_nat = None
    for fc in range(nfc):
        h_next = [None] * nsl
        for sl in range(nsl):
            if fc + 1 < nfc:
                h_next[sl] = hidden(fc + 1, sl)
            else:
                if sl == 0:
                    q_carry()
                    o_nat = ot_ref[...].reshape(D, TQ).T.astype(BF16)
                a[sl] = _dot(o_nat[sl * SL:(sl + 1) * SL, :], wo_ref[...])
            if fc == 0 and sl == 0:
                q_store(qt, hs)
            bb = _dot(h_prev[sl], wd_ref[fc * FC:(fc + 1) * FC, :])
            b[sl] = bb if b[sl] is None else b[sl] + bb
        h_prev = h_next
    a = jnp.concatenate(a, axis=0)
    b = jnp.concatenate(b, axis=0)
    logit = jnp.sum(xb.astype(F32) * gw_ref[...].astype(F32).reshape(1, D),
                    axis=1, keepdims=True)
    g = 1.0 / (1.0 + jnp.exp(-logit))
    o_ref[0] = (g * a + (1.0 - g) * b).astype(o_ref.dtype)


@jax.jit
def pallas_gated_mix__grouped_kv_mqa__glu_gated_reglu__prompt_kernel(
    A_x: jax.Array,
    A_wq: jax.Array,
    A_wk: jax.Array,
    A_wv: jax.Array,
    A_wo: jax.Array,
    B_x: jax.Array,
    B_W_gate: jax.Array,
    B_W_up: jax.Array,
    B_W_down: jax.Array,
    gate_w: jax.Array,
):
    del B_x
    hbm = pl.BlockSpec(memory_space=pl.ANY)

    return pl.pallas_call(
        _kernel,
        grid=(NBLK,),
        in_specs=[hbm] * 9,
        out_specs=pl.BlockSpec((1, TQ, D), lambda i: (0, i, 0)),
        out_shape=jax.ShapeDtypeStruct((1, S, D), BF16),
        scratch_shapes=[
            pltpu.VMEM((S, D), BF16),
            pltpu.VMEM((D, D), BF16),
            pltpu.VMEM((DH, D), BF16),
            pltpu.VMEM((DH, D), BF16),
            pltpu.VMEM((D, D), BF16),
            pltpu.VMEM((D, F), BF16),
            pltpu.VMEM((D, F), BF16),
            pltpu.VMEM((F, D), BF16),
            pltpu.VMEM((D,), BF16),
            pltpu.VMEM((S // 2, 128), jnp.uint32),
            pltpu.VMEM((VR, S), F32),
            pltpu.VMEM((NP, 2, KD // 2, TQ), jnp.uint32),
            pltpu.VMEM((SC, TQ), F32),
            pltpu.VMEM((NP, 2 * DH, TQ), F32),
            pltpu.VMEM((128, D), F32),
            pltpu.VMEM((TQ, D), F32),
            pltpu.VMEM((DH, NVK, 128), F32),
            pltpu.VMEM((NP, 2 * DH, TQ), F32),
            pltpu.SMEM((1,), F32),
            pltpu.SMEM((1,), F32),
            pltpu.SMEM((1,), jnp.int32),
            pltpu.SMEM((NZ,), jnp.int32),
            pltpu.SemaphoreType.DMA((NBLK + 8,)),
        ],
        compiler_params=pltpu.CompilerParams(
            dimension_semantics=("arbitrary",),
            vmem_limit_bytes=100 * 1024 * 1024,
        ),
    )(A_x.reshape(S, D), A_wq, A_wk.T, A_wv.T, A_wo, B_W_gate, B_W_up, B_W_down, gate_w)
```

```python
import jax
import jax.numpy as jnp
from jax import lax
from jax.experimental import pallas as pl
from jax.experimental.pallas import tpu as pltpu

S = 2048
D = 640
H = 32
DH = 20
F = 1536
TQ = 512
NBLK = S // TQ
CK = 128
NCK = S // CK
SC = 256
NSC = S // SC
VRS = [0] + [16] * (NSC - 1)
VOFF = [sum(VRS[:c]) for c in range(NSC)]
NVK = sum(VRS)
GR = 16
GL = 256
NP = H // 2
UNROLL = 4
KD = 32
VR = 24
FC = 512
SL = 256
NZ = 64
LOG2E = 1.4426950408889634
QSCALE = (DH ** -0.5) * LOG2E
SAFE_M = 16.0

F32 = jnp.float32
BF16 = jnp.bfloat16


def _dot(a, b):
    return jnp.dot(a, b, preferred_element_type=F32)


def _pk(x):
    return pltpu.bitcast(x, jnp.uint32)


def _unpk(x):
    return pltpu.bitcast(x, BF16)


def _rev8(p):
    n = p.shape[0] // 8
    return jnp.concatenate([p[8 * (n - 1 - t):8 * (n - t)] for t in range(n)], axis=0)


def _kernel(x_hbm, wq_hbm, wkt_hbm, wvt_hbm, wo_hbm, wg_hbm, wu_hbm, wd_hbm, gw_hbm,
            o_ref,
            x_ref, wq_ref, wkt_ref, wvt_ref, wo_ref, wg_ref, wu_ref, wd_ref, gw_ref,
            k_ref, vt_ref, qw_ref, carry_ref, ot_ref, wt_ref, q_ref,
            kb_ref, qf_ref, kn_ref, m_ref, flag_ref, z_ref, sems):
    step = pl.program_id(0)

    def x_copy(c):
        return pltpu.make_async_copy(x_hbm.at[pl.ds(c * TQ, TQ)],
                                     x_ref.at[pl.ds(c * TQ, TQ)], sems.at[c])

    early = [pltpu.make_async_copy(wq_hbm, wq_ref, sems.at[NBLK]),
             pltpu.make_async_copy(wkt_hbm, wkt_ref, sems.at[NBLK + 1]),
             pltpu.make_async_copy(wvt_hbm, wvt_ref, sems.at[NBLK + 2])]
    late = [pltpu.make_async_copy(wo_hbm, wo_ref, sems.at[NBLK + 3]),
            pltpu.make_async_copy(wg_hbm, wg_ref, sems.at[NBLK + 4]),
            pltpu.make_async_copy(wu_hbm, wu_ref, sems.at[NBLK + 5]),
            pltpu.make_async_copy(wd_hbm, wd_ref, sems.at[NBLK + 6]),
            pltpu.make_async_copy(gw_hbm, gw_ref, sems.at[NBLK + 7])]

    def k_rows(r0, n):
        return _unpk(k_ref[r0 // 2:(r0 + n) // 2, :])[:, 0:KD]

    def q_bcast(j, par):
        return [jnp.broadcast_to(qf_ref[j, par * DH + d:par * DH + d + 1, :], (8, TQ))
                for d in range(DH)]

    def probs(j, par, c, g, qbs):
        s = _dot(k_rows(c * SC, SC - VRS[c]), _unpk(qw_ref[j + z_ref[g % NZ], par]))
        vrows = []
        for gg in range(VRS[c] // GR):
            r0 = VOFF[c] + gg * GR
            lanes = []
            for ll in range(TQ // GL):
                zi = z_ref[(g * 8 + gg * (TQ // GL) + ll + 7) % NZ]
                a = jnp.full((GR, GL), m_ref[0], F32)
                for d in range(DH):
                    kb = kb_ref[d + zi, r0:r0 + GR, :]
                    kb = jnp.concatenate([kb] * (GL // 128), axis=1)
                    qb = qbs[d][:, ll * GL:(ll + 1) * GL]
                    qb = jnp.concatenate([qb] * (GR // 8), axis=0)
                    a = a + kb * qb
                parts = [a[rr * 8:(rr + 1) * 8, lq * 128:(lq + 1) * 128]
                         for rr in range(GR // 8) for lq in range(GL // 128)]
                t = parts[0]
                for part in parts[1:]:
                    t = t + part
                t = t * 0.0
                t = jnp.concatenate([t] * (GL // 128), axis=1)
                t = jnp.concatenate([t] * (GR // 8), axis=0)
                lanes.append(jnp.exp2(a + t))
            vrows.append(jnp.concatenate(lanes, axis=1))
        p = jnp.concatenate([jnp.exp2(s)] + vrows, axis=0)
        return jnp.concatenate(
            [_rev8(p[t0:t0 + CK]) for t0 in range(0, SC, CK)], axis=0)

    def q_raw(blk):
        r0 = pl.multiple_of(blk * TQ, TQ)
        return _dot(x_ref[pl.ds(r0, TQ), :], wq_ref[...]) * QSCALE

    def q_norms(qt):
        sq = (qt * qt).astype(BF16)
        hrow = lax.broadcasted_iota(jnp.int32, (H, D), 0)
        hcol = lax.broadcasted_iota(jnp.int32, (H, D), 1)
        e = jnp.logical_and(hcol >= hrow * DH, hcol < (hrow + 1) * DH)
        return _dot(jnp.where(e, 1.0, 0.0).astype(BF16), sq)

    def q_store(qt, hs):
        m2 = jnp.max(hs) * kn_ref[0] * 1.05
        safe = m2 <= SAFE_M * SAFE_M
        flag_ref[0] = safe.astype(jnp.int32)
        mval = jnp.where(safe, -jnp.sqrt(jnp.full((KD - DH, TQ), m2, F32)), 0.0)
        srow = lax.broadcasted_iota(jnp.int32, (KD - DH, TQ), 0)
        mt = jnp.where(srow == 0, mval, 0.0)
        for h in range(H):
            qw_ref[h // 2, h % 2] = _pk(jnp.concatenate(
                [qt[h * DH:(h + 1) * DH, :], mt], axis=0).astype(BF16))
        m_ref[0] = jnp.min(mt.astype(BF16).astype(F32))
        qf_ref[...] = qt.astype(BF16).astype(F32).reshape(NP, 2 * DH, TQ)

    def q_carry():
        carry_ref[...] = probs(0, 0, 0, 5, q_bcast(0, 0))

    @pl.when(step == 0)
    def _init():
        x_copy(0).start()
        early[1].start()
        early[2].start()
        early[0].start()
        for c in range(1, NBLK):
            x_copy(c).start()
        wt_ref[...] = jnp.zeros_like(wt_ref)
        for i in range(NZ):
            z_ref[i] = 0
        early[1].wait()
        early[2].wait()
        wt_ref[0:DH, :] = wkt_ref[...].astype(F32)
        wt_ref[64:64 + DH, :] = wvt_ref[...].astype(F32)
        wall = wt_ref[...].T.astype(BF16)
        lane = lax.broadcasted_iota(jnp.int32, (TQ, 128), 1)
        vrow = lax.broadcasted_iota(jnp.int32, (VR, CK), 0)
        k_fill = jnp.where(lane == DH, 1.0, 0.0)

        def kv(c, kn):
            rows = slice(c * TQ, (c + 1) * TQ)
            r = _dot(x_ref[rows, :], wall)
            r = r.astype(BF16).astype(F32)
            k_ref[c * TQ // 2:(c + 1) * TQ // 2, :] = _pk(
                jnp.where(lane < DH, r, k_fill).astype(BF16))
            for u in range(TQ // SC):
                sc = c * (TQ // SC) + u
                if VRS[sc]:
                    rv = r[(u + 1) * SC - VRS[sc]:(u + 1) * SC, :]
                    for d in range(DH):
                        kb_ref[d, VOFF[sc]:VOFF[sc] + VRS[sc], :] = jnp.broadcast_to(
                            rv[:, d:d + 1], (VRS[sc], 128))
            for t in range(TQ // CK):
                rt = _rev8(r[t * CK:(t + 1) * CK, :]).T
                col = c * TQ + t * CK
                vt_ref[:, col:col + CK] = jnp.where(
                    vrow < DH, rt[64:64 + VR, :], jnp.where(vrow == DH, 1.0, 0.0))
                kt = rt[0:DH, :]
                n2 = jnp.sum(kt * kt, axis=0, keepdims=True)
                kn = n2 if kn is None else jnp.maximum(kn, n2)
            return kn

        x_copy(0).wait()
        kn = kv(0, None)
        early[0].wait()
        q_ref[...] = q_raw(0)
        for c in range(1, NBLK):
            x_copy(c).wait()
        for cp in late:
            cp.start()
        for c in range(1, NBLK):
            kn = kv(c, kn)
        kn_ref[0] = jnp.max(kn)
        qt0 = q_ref[...].T
        q_store(qt0, q_norms(qt0))
        q_carry()

    def finish(acc):
        return acc[0:DH, :] * (1.0 / acc[DH:DH + 1, :])

    @pl.when(flag_ref[0] == 1)
    def _fast():
        def body(i, carry):
            j0 = i * UNROLL
            pend = carry_ref[...]
            acc = None
            n = UNROLL * 2 * NSC
            for g in range(n):
                gq = g + 1
                if gq < n:
                    jq, pq = j0 + gq // (2 * NSC), (gq // NSC) % 2
                    if gq % NSC == 0 or g == 0:
                        qbs = q_bcast(jq, pq)
                    nxt = probs(jq, pq, gq % NSC, g, qbs)
                else:
                    jq = jnp.minimum(j0 + UNROLL, NP - 1)
                    nxt = probs(jq, 0, 0, g, q_bcast(jq, 0))
                c = g % NSC
                o = _dot(vt_ref[:, c * SC:(c + 1) * SC], pend)
                acc = o if c == 0 else acc + o
                if c == NSC - 1:
                    par = (g // NSC) % 2
                    ot_ref[j0 + g // (2 * NSC), par * DH:(par + 1) * DH, :] = finish(acc)
                pend = nxt
            carry_ref[...] = pend
            return carry

        lax.fori_loop(0, NP // UNROLL, body, 0)

    @pl.when(flag_ref[0] != 1)
    def _slow():
        def head(j, par, s_ref):
            qw = _unpk(qw_ref[j, par])
            m = None
            for c in range(NCK):
                s = _dot(k_rows(c * CK, CK), qw)
                s_ref[c * CK:(c + 1) * CK, :] = s
                mc = jnp.max(s, axis=0, keepdims=True)
                m = mc if m is None else jnp.maximum(m, mc)
            acc = None
            for c in range(NCK):
                p = _rev8(jnp.exp2(s_ref[c * CK:(c + 1) * CK, :] - m))
                o = _dot(vt_ref[:, c * CK:(c + 1) * CK], p)
                acc = o if acc is None else acc + o
            ot_ref[j, par * DH:(par + 1) * DH, :] = finish(acc)

        def scoped(s_ref):
            def body(j, carry):
                head(j, 0, s_ref)
                head(j, 1, s_ref)
                return carry
            lax.fori_loop(0, NP, body, 0)

        pl.run_scoped(scoped, pltpu.VMEM((S, TQ), F32))

    @pl.when(step == 0)
    def _wait_late():
        for cp in late:
            cp.wait()

    @pl.when(step < NBLK - 1)
    def _next_q():
        q_ref[...] = q_raw(step + 1)

    r0 = pl.multiple_of(step * TQ, TQ)
    xb = x_ref[pl.ds(r0, TQ), :]
    nsl = TQ // SL
    nfc = F // FC

    def hidden(fc, sl):
        xs = xb[sl * SL:(sl + 1) * SL, :]
        gt = _dot(xs, wg_ref[:, fc * FC:(fc + 1) * FC])
        up = _dot(xs, wu_ref[:, fc * FC:(fc + 1) * FC])
        return (jnp.maximum(gt, 0.0) * up).astype(BF16)

    h_prev = [hidden(0, sl) for sl in range(nsl)]
    qt = q_ref[...].T
    hs = q_norms(qt)
    logit = jnp.sum(xb.astype(F32) * gw_ref[...].astype(F32).reshape(1, D),
                    axis=1, keepdims=True)
    g = 1.0 / (1.0 + jnp.exp(-logit))
    b = [None] * nsl
    o_nat = None
    for fc in range(nfc):
        h_next = [None] * nsl
        for sl in range(nsl):
            rows = slice(sl * SL, (sl + 1) * SL)
            if fc + 1 < nfc:
                h_next[sl] = hidden(fc + 1, sl)
            else:
                if sl == 0:
                    o_nat = ot_ref[...].reshape(D, TQ).T.astype(BF16)
                a = _dot(o_nat[rows, :], wo_ref[...])
            if fc == 0 and sl == 0:
                q_store(qt, hs)
            bb = _dot(h_prev[sl], wd_ref[fc * FC:(fc + 1) * FC, :])
            b[sl] = bb if b[sl] is None else b[sl] + bb
            if fc + 1 == nfc:
                gs = g[rows, :]
                o_ref[0, rows, :] = (gs * a + (1.0 - gs) * b[sl]).astype(o_ref.dtype)
        h_prev = h_next
    q_carry()


@jax.jit
def pallas_gated_mix__grouped_kv_mqa__glu_gated_reglu__prompt_kernel(
    A_x: jax.Array,
    A_wq: jax.Array,
    A_wk: jax.Array,
    A_wv: jax.Array,
    A_wo: jax.Array,
    B_x: jax.Array,
    B_W_gate: jax.Array,
    B_W_up: jax.Array,
    B_W_down: jax.Array,
    gate_w: jax.Array,
):
    del B_x
    hbm = pl.BlockSpec(memory_space=pl.ANY)

    return pl.pallas_call(
        _kernel,
        grid=(NBLK,),
        in_specs=[hbm] * 9,
        out_specs=pl.BlockSpec((1, TQ, D), lambda i: (0, i, 0)),
        out_shape=jax.ShapeDtypeStruct((1, S, D), BF16),
        scratch_shapes=[
            pltpu.VMEM((S, D), BF16),
            pltpu.VMEM((D, D), BF16),
            pltpu.VMEM((DH, D), BF16),
            pltpu.VMEM((DH, D), BF16),
            pltpu.VMEM((D, D), BF16),
            pltpu.VMEM((D, F), BF16),
            pltpu.VMEM((D, F), BF16),
            pltpu.VMEM((F, D), BF16),
            pltpu.VMEM((D,), BF16),
            pltpu.VMEM((S // 2, 128), jnp.uint32),
            pltpu.VMEM((VR, S), F32),
            pltpu.VMEM((NP, 2, KD // 2, TQ), jnp.uint32),
            pltpu.VMEM((SC, TQ), F32),
            pltpu.VMEM((NP, 2 * DH, TQ), F32),
            pltpu.VMEM((128, D), F32),
            pltpu.VMEM((TQ, D), F32),
            pltpu.VMEM((DH, NVK, 128), F32),
            pltpu.VMEM((NP, 2 * DH, TQ), F32),
            pltpu.SMEM((1,), F32),
            pltpu.SMEM((1,), F32),
            pltpu.SMEM((1,), jnp.int32),
            pltpu.SMEM((NZ,), jnp.int32),
            pltpu.SemaphoreType.DMA((NBLK + 8,)),
        ],
        compiler_params=pltpu.CompilerParams(
            dimension_semantics=("arbitrary",),
            vmem_limit_bytes=100 * 1024 * 1024,
        ),
    )(A_x.reshape(S, D), A_wq, A_wk.T, A_wv.T, A_wo, B_W_gate, B_W_up, B_W_down, gate_w)
```
